```python
import jax
import jax.numpy as jnp

def _softmax(x, axis=-1):
    return jax.nn.softmax(x, axis=axis)
def _gelu(x):
    return jax.nn.gelu(x, approximate=True)
def _silu(x):
    return jax.nn.silu(x)
def _sigmoid(x):
    return jax.nn.sigmoid(x)
def _layernorm(x, axis=-1, eps=1e-5):
    m = jnp.mean(x, axis=axis, keepdims=True)
    v = jnp.var(x, axis=axis, keepdims=True)
    return (x - m) / jnp.sqrt(v + eps)
def _scatter_add(tgt, idx, src, axis=0):
    return tgt.at[idx].add(src)
def _segment_sum(src, seg, n):
    return jax.ops.segment_sum(src, seg, n)
class _Rng:
    def __init__(self, key):
        self._k = key
    def _next(self):
        self._k, sub = jax.random.split(self._k)
        return sub
    def normal(self, shape):
        return jax.random.normal(self._next(), shape, dtype=jnp.bfloat16)
    def randint(self, lo, hi, shape):
        return jax.random.randint(self._next(), shape, lo, hi, dtype=jnp.int32)
    def uniform(self, shape, lo=0.0, hi=1.0):
        return jax.random.uniform(self._next(), shape, jnp.bfloat16, lo, hi)
    def permutation(self, n):
        return jax.random.permutation(self._next(), n)


kernel_name = 'standalone__instancenorm__prompt'

def setup_inputs():
    _rng = _Rng(jax.random.key(int.from_bytes(__import__("os").urandom(4), "little")))
    _w = (lambda a: (lambda t: t.astype(jnp.bfloat16) if jnp.issubdtype(t.dtype, jnp.floating) else t)(jnp.asarray(a)))
    B, C, H, W = 2, 1024, 2048, 32
    return {
        "x": _w((lambda *s: _rng.normal(s) * 0.05)(B, C, H, W)),
        "g": _w((lambda *s: _rng.normal(s) * 0.05)(C) + 1.0),
        "b": _w((lambda *s: _rng.normal(s) * 0.05)(C)),
    }

def reference(x, g, b):
    mu = x.mean(axis=(-2, -1), keepdims=True)
    var = ((x - mu) * (x - mu)).mean(axis=(-2, -1), keepdims=True)
    xhat = (x - mu) / jnp.sqrt(var + 1e-5)
    return xhat * g.reshape(1, -1, 1, 1) + b.reshape(1, -1, 1, 1)
```

```python
import jax
import jax.numpy as jnp
import jax.experimental.pallas as pl
import jax.experimental.pallas.tpu as pltpu

_EPS = 1e-5
_ROWS = 8
_S = 16
_M = 32
_W = 4
_NL = 2
_CS = 2
_DR = 4
_DW = 8
_U = 2
_NACC = 4


def _tree_sum(vs):
    vs = list(vs)
    while len(vs) > 1:
        nxt = [vs[i] + vs[i + 1] for i in range(0, len(vs) - 1, 2)]
        if len(vs) % 2:
            nxt.append(vs[-1])
        vs = nxt
    return vs[0]


def _make_kernel(n_inst, n_ch, ppc, L):
    f32 = jnp.float32
    S, M, W, NL, CS, DR, DW, U = _S, _M, _W, _NL, _CS, _DR, _DW, _U
    LL = L // NL
    cpr = M // ppc
    P = W * S * cpr
    assert n_inst % P == 0
    n_phase = n_inst // P
    G = CS * cpr
    K = W * S // CS
    NW = W * M * NL
    inv_n = 1.0 / (ppc * _ROWS * L)

    def kernel(x_hbm, g_ref, b_ref, o_hbm,
               buf, part, st_mu, st_a, st_s, gb_vmem, gb_smem, rsem, wsem, gsem):
        def rd(p, j):
            w, s = (j * CS) // S, (j * CS) % S
            return pltpu.make_async_copy(
                x_hbm.at[p * W + w, pl.ds(s, CS)], buf.at[w, pl.ds(s, CS)],
                rsem.at[j % DR])

        def wr(p, i):
            l, i2 = i % NL, i // NL
            w, m = i2 // M, i2 % M
            ls = pl.ds(pl.multiple_of(l * LL, 128), LL)
            return pltpu.make_async_copy(
                buf.at[w, :, m, :, ls], o_hbm.at[p * W + w, :, m, :, ls],
                wsem.at[i % DW])

        for j in range(DR):
            rd(0, j).start()

        gb_vmem[0] = g_ref[...].astype(f32)
        gb_vmem[1] = b_ref[...].astype(f32)
        cp = pltpu.make_async_copy(gb_vmem, gb_smem, gsem)
        cp.start()
        cp.wait()

        def loc(j, c):
            sr = j * CS + c // cpr
            return sr // S, sr % S, (c % cpr) * ppc

        def load(w, s, m):
            v = buf[w, s, m].astype(f32)
            return [v[:, t * 128:(t + 1) * 128] for t in range(L // 128)]

        def full_sum(v):
            return jnp.sum(jnp.sum(v, axis=1, keepdims=True), axis=2, keepdims=True)

        def compute_chunk(p, j):
            def pass_mean(ci, carry):
                for u in range(U):
                    c = ci * U + u
                    w, s, m0 = loc(j, c)
                    part[c] = _tree_sum(
                        [_tree_sum(load(w, s, m0 + r)) for r in range(ppc)])
                return carry
            jax.lax.fori_loop(0, G // U, pass_mean, 0)
            st_mu[...] = jnp.broadcast_to(full_sum(part[...]) * inv_n, st_mu.shape)

            def pass_var(ci, carry):
                for u in range(U):
                    c = ci * U + u
                    w, s, m0 = loc(j, c)
                    mu = st_mu[c]
                    accs = [None] * _NACC
                    t = 0
                    for r in range(ppc):
                        for v in load(w, s, m0 + r):
                            d = v - mu
                            d = d * d
                            a = accs[t % _NACC]
                            accs[t % _NACC] = d if a is None else a + d
                            t += 1
                    part[c] = _tree_sum(accs)
                return carry
            jax.lax.fori_loop(0, G // U, pass_var, 0)
            var = full_sum(part[...]) * inv_n
            rstd = jnp.broadcast_to(jax.lax.rsqrt(var + _EPS), st_a.shape)

            ch0 = p * P + j * G
            for c in range(G):
                ch = (ch0 + c) % n_ch
                a = rstd[c] * gb_smem[0, ch // 128, ch % 128]
                st_a[c] = a
                st_s[c] = gb_smem[1, ch // 128, ch % 128] - st_mu[c] * a

            def pass_norm(ci, carry):
                for u in range(U):
                    c = ci * U + u
                    w, s, m0 = loc(j, c)
                    a = jnp.concatenate([st_a[c]] * (L // 128), axis=1)
                    sh = jnp.concatenate([st_s[c]] * (L // 128), axis=1)
                    for r in range(ppc):
                        v = buf[w, s, m0 + r].astype(f32)
                        buf[w, s, m0 + r] = (v * a + sh).astype(buf.dtype)
                return carry
            jax.lax.fori_loop(0, G // U, pass_norm, 0)

        def phase(p, carry):
            def chunk(j, carry):
                rd(p, j).wait()

                @pl.when(j + DR < K)
                def _():
                    rd(p, j + DR).start()

                @pl.when(j == K - 1)
                def _():
                    for i in range(DW):
                        wr(p, i).start()

                compute_chunk(p, j)
                return carry
            jax.lax.fori_loop(0, K, chunk, 0)

            def drain(i, carry):
                wr(p, i).wait()

                @pl.when(i + DW < NW)
                def _():
                    wr(p, i + DW).start()
                return carry
            jax.lax.fori_loop(0, NW, drain, 0)

            @pl.when(p + 1 < n_phase)
            def _():
                for j in range(DR):
                    rd(p + 1, j).start()
            return carry
        jax.lax.fori_loop(0, n_phase, phase, 0)

    scratch = [
        pltpu.VMEM((W, S, M, _ROWS, L), jnp.bfloat16),
        pltpu.VMEM((G, 8, 128), f32),
        pltpu.VMEM((G, 8, 128), f32),
        pltpu.VMEM((G, 8, 128), f32),
        pltpu.VMEM((G, 8, 128), f32),
        pltpu.VMEM((2, n_ch // 128, 128), f32),
        pltpu.SMEM((2, n_ch // 128, 128), f32),
        pltpu.SemaphoreType.DMA((DR,)),
        pltpu.SemaphoreType.DMA((DW,)),
        pltpu.SemaphoreType.DMA,
    ]
    return kernel, scratch


@jax.jit
def pallas_standalone__instancenorm__prompt_kernel(
    x: jax.Array,
    g: jax.Array,
    b: jax.Array,
):
    B, C, H, Wd = x.shape
    assert Wd % _ROWS == 0 and H % 128 == 0 and C % 128 == 0
    ppc = Wd // _ROWS
    n_pieces = B * C * ppc
    kernel, scratch = _make_kernel(B * C, C, ppc, H)
    xt = x.transpose(0, 1, 3, 2).reshape(n_pieces // (_S * _M), _S, _M, _ROWS, H)
    out = pl.pallas_call(
        kernel,
        in_specs=[
            pl.BlockSpec(memory_space=pl.ANY),
            pl.BlockSpec((C // 128, 128), lambda: (0, 0)),
            pl.BlockSpec((C // 128, 128), lambda: (0, 0)),
        ],
        out_specs=pl.BlockSpec(memory_space=pl.ANY),
        out_shape=jax.ShapeDtypeStruct(xt.shape, x.dtype),
        scratch_shapes=scratch,
        compiler_params=pltpu.CompilerParams(vmem_limit_bytes=100 * 1024 * 1024),
    )(xt, g.reshape(C // 128, 128), b.reshape(C // 128, 128))
    return out.reshape(B, C, Wd, H).transpose(0, 1, 3, 2)
```

```python
import jax
import jax.numpy as jnp
import jax.experimental.pallas as pl
import jax.experimental.pallas.tpu as pltpu

_EPS = 1e-5
_ROWS = 8
_S = 16
_M = 32
_PHASES = (6, 5, 5)
_NL = 2
_CS = 2
_DR = 6
_DW = 64
_LAG = 5
_U = 4
_NACC = 4


def _tree_sum(vs):
    vs = list(vs)
    while len(vs) > 1:
        nxt = [vs[i] + vs[i + 1] for i in range(0, len(vs) - 1, 2)]
        if len(vs) % 2:
            nxt.append(vs[-1])
        vs = nxt
    return vs[0]


def _select(p, vals):
    r = jnp.int32(vals[0])
    for i in range(1, len(vals)):
        r = jnp.where(p == i, vals[i], r)
    return r


def _make_kernel(n_groups, n_ch, ppc, L):
    f32 = jnp.float32
    S, M, NL, CS, DR, DW, LAG, U = _S, _M, _NL, _CS, _DR, _DW, _LAG, _U
    LL = L // NL
    cpr = M // ppc
    G = CS * cpr
    kpg = S // CS
    wpg = M * NL
    n_phase = len(_PHASES)
    first = [sum(_PHASES[:i]) for i in range(n_phase)]
    assert sum(_PHASES) == n_groups and M % ppc == 0 and G % U == 0
    assert LAG <= DR and DW <= wpg and min(_PHASES) * kpg - LAG >= kpg
    inv_n = 1.0 / (ppc * _ROWS * L)

    def kernel(x_hbm, g_ref, b_ref, o_hbm,
               buf, part, st_mu, st_a, st_b, gb_vmem, gb_smem, rsem, wsem, gsem):
        def rd_start(g0, j):
            t = 0
            for ss in range(CS):
                sr = j * CS + ss
                w, s = sr // S, sr % S
                for i in range(cpr):
                    sl = pl.ds(i * ppc, ppc)
                    pltpu.make_async_copy(
                        x_hbm.at[g0 + w, s, sl], buf.at[w, s, sl],
                        rsem.at[j % DR]).start(priority=t % 2)
                    t += 1

        def rd_wait(j):
            d = buf.at[(j * CS) // S, pl.ds((j * CS) % S, CS)]
            pltpu.make_async_copy(d, d, rsem.at[j % DR]).wait()

        def wr(g0, i):
            l, i2 = i % NL, i // NL
            w, m = i2 // M, i2 % M
            ls = pl.ds(pl.multiple_of(l * LL, 128), LL)
            return pltpu.make_async_copy(
                buf.at[w, :, m, :, ls], o_hbm.at[g0 + w, :, m, :, ls],
                wsem.at[i % DW])

        for j in range(DR):
            rd_start(0, j)

        gb_vmem[0] = g_ref[...].astype(f32)
        gb_vmem[1] = b_ref[...].astype(f32)
        cp = pltpu.make_async_copy(gb_vmem, gb_smem, gsem)
        cp.start()
        cp.wait()

        def loc(j, c):
            sr = j * CS + c // cpr
            return sr // S, sr % S, (c % cpr) * ppc

        def load(w, s, m):
            v = buf[w, s, m].astype(f32)
            return [v[:, t * 128:(t + 1) * 128] for t in range(L // 128)]

        def full_sum(v):
            return jnp.sum(jnp.sum(v, axis=1, keepdims=True), axis=2, keepdims=True)

        def wide(v):
            return jnp.concatenate([v] * (L // 128), axis=1)

        def compute_chunk(g0, j):
            def pass_mean(ci, carry):
                for u in range(U):
                    c = ci * U + u
                    w, s, m0 = loc(j, c)
                    part[c] = _tree_sum(
                        [_tree_sum(load(w, s, m0 + r)) for r in range(ppc)])
                return carry
            jax.lax.fori_loop(0, G // U, pass_mean, 0)
            st_mu[...] = jnp.broadcast_to(full_sum(part[...]) * inv_n, st_mu.shape)

            def pass_var(ci, carry):
                for u in range(U):
                    c = ci * U + u
                    w, s, m0 = loc(j, c)
                    mu = st_mu[c]
                    accs = [None] * _NACC
                    t = 0
                    for r in range(ppc):
                        for v in load(w, s, m0 + r):
                            d = v - mu
                            d = d * d
                            a = accs[t % _NACC]
                            accs[t % _NACC] = d if a is None else a + d
                            t += 1
                    part[c] = _tree_sum(accs)
                return carry
            jax.lax.fori_loop(0, G // U, pass_var, 0)
            var = full_sum(part[...]) * inv_n
            rstd = jnp.broadcast_to(jax.lax.rsqrt(var + _EPS), st_a.shape)

            ch0 = g0 * S * cpr + j * G
            for c in range(G):
                ch = (ch0 + c) % n_ch
                st_a[c] = rstd[c] * gb_smem[0, ch // 128, ch % 128]
                st_b[c] = jnp.full((8, 128), gb_smem[1, ch // 128, ch % 128], f32)

            def pass_norm(ci, carry):
                for u in range(U):
                    c = ci * U + u
                    w, s, m0 = loc(j, c)
                    mu, a, b = wide(st_mu[c]), wide(st_a[c]), wide(st_b[c])
                    for r in range(ppc):
                        v = buf[w, s, m0 + r].astype(f32)
                        buf[w, s, m0 + r] = ((v - mu) * a + b).astype(buf.dtype)
                return carry
            jax.lax.fori_loop(0, G // U, pass_norm, 0)

        def phase(p, carry):
            n_grp, g0 = _select(p, _PHASES), _select(p, first)
            K, NW = n_grp * kpg, n_grp * wpg
            j_hand = K - LAG

            def chunk(j, carry):
                @pl.when(j < j_hand)
                def _():
                    rd_wait(j)

                    @pl.when(j + DR < K)
                    def _():
                        rd_start(g0, j + DR)

                @pl.when(j == j_hand)
                def _():
                    for t in range(LAG - 1):
                        rd_wait(j + t)

                    def start(i, carry):
                        wr(g0, i).start()
                        return carry
                    jax.lax.fori_loop(0, DW, start, 0)
                    rd_wait(j + LAG - 1)

                compute_chunk(g0, j)
                return carry
            jax.lax.fori_loop(0, K, chunk, 0)

            def drain(i, carry):
                wr(g0, i).wait()

                @pl.when(i + DW < NW)
                def _():
                    wr(g0, i + DW).start()
                return carry
            jax.lax.fori_loop(0, NW, drain, 0)

            @pl.when(p + 1 < n_phase)
            def _():
                for j in range(DR):
                    rd_start(g0 + n_grp, j)
            return carry
        jax.lax.fori_loop(0, n_phase, phase, 0)

    scratch = [
        pltpu.VMEM((max(_PHASES), S, M, _ROWS, L), jnp.bfloat16),
        pltpu.VMEM((G, 8, 128), f32),
        pltpu.VMEM((G, 8, 128), f32),
        pltpu.VMEM((G, 8, 128), f32),
        pltpu.VMEM((G, 8, 128), f32),
        pltpu.VMEM((2, n_ch // 128, 128), f32),
        pltpu.SMEM((2, n_ch // 128, 128), f32),
        pltpu.SemaphoreType.DMA((DR,)),
        pltpu.SemaphoreType.DMA((DW,)),
        pltpu.SemaphoreType.DMA,
    ]
    return kernel, scratch


@jax.jit
def pallas_standalone__instancenorm__prompt_kernel(
    x: jax.Array,
    g: jax.Array,
    b: jax.Array,
):
    B, C, H, Wd = x.shape
    assert Wd % _ROWS == 0 and H % (128 * _NL) == 0 and C % 128 == 0
    ppc = Wd // _ROWS
    n_groups = B * C * ppc // (_S * _M)
    kernel, scratch = _make_kernel(n_groups, C, ppc, H)
    xt = x.transpose(0, 1, 3, 2).reshape(n_groups, _S, _M, _ROWS, H)
    out = pl.pallas_call(
        kernel,
        in_specs=[
            pl.BlockSpec(memory_space=pl.ANY),
            pl.BlockSpec((C // 128, 128), lambda: (0, 0)),
            pl.BlockSpec((C // 128, 128), lambda: (0, 0)),
        ],
        out_specs=pl.BlockSpec(memory_space=pl.ANY),
        out_shape=jax.ShapeDtypeStruct(xt.shape, x.dtype),
        scratch_shapes=scratch,
        compiler_params=pltpu.CompilerParams(vmem_limit_bytes=104 * 1024 * 1024),
    )(xt, g.reshape(C // 128, 128), b.reshape(C // 128, 128))
    return out.reshape(B, C, Wd, H).transpose(0, 1, 3, 2)
```
